```python
import jax
import jax.numpy as jnp

def _softmax(x, axis=-1):
    return jax.nn.softmax(x, axis=axis)

def _gelu(x):
    return jax.nn.gelu(x, approximate=True)

def _silu(x):
    return jax.nn.silu(x)

def _sigmoid(x):
    return jax.nn.sigmoid(x)

def _layernorm(x, axis=-1, eps=1e-05):
    m = jnp.mean(x, axis=axis, keepdims=True)
    v = jnp.var(x, axis=axis, keepdims=True)
    return (x - m) / jnp.sqrt(v + eps)

def _scatter_add(tgt, idx, src, axis=0):
    return tgt.at[idx].add(src)

def _segment_sum(src, seg, n):
    return jax.ops.segment_sum(src, seg, n)

class _Rng:

    def __init__(self, key):
        self._k = key

    def _next(self):
        self._k, sub = jax.random.split(self._k)
        return sub

    def normal(self, shape):
        return jax.random.normal(self._next(), shape, dtype=jnp.bfloat16)

    def randint(self, lo, hi, shape):
        return jax.random.randint(self._next(), shape, lo, hi, dtype=jnp.int32)

    def uniform(self, shape, lo=0.0, hi=1.0):
        return jax.random.uniform(self._next(), shape, jnp.bfloat16, lo, hi)

    def permutation(self, n):
        return jax.random.permutation(self._next(), n)
kernel_name = 'adaLN_cond__sliding_block_cached__geglu_ffn__decode'

def setup_inputs():
    _rng = _Rng(jax.random.key(int.from_bytes(__import__("os").urandom(4), "little")))
    _w = lambda a: (lambda t: t.astype(jnp.bfloat16) if jnp.issubdtype(t.dtype, jnp.floating) else t)(jnp.asarray(a))

    def _A_setup():
        B, Sq, D = (1, 1, 640)
        Hq, Hkv, Sk, Dh = (32, 32, 32768, 192)
        assert Hq % Hkv == 0, (Hq, Hkv)
        return {'x': _w((lambda *s: _rng.normal(s) * 0.05)(B, Sq, D)), 'k_cache': _w((lambda *s: _rng.normal(s) * 0.05)(B, Hkv, Sk, Dh)), 'v_cache': _w((lambda *s: _rng.normal(s) * 0.05)(B, Hkv, Sk, Dh)), 'wq': _w((lambda *s: _rng.normal(s) * 0.05)(D, Hq * Dh) * D ** (-0.5)), 'wo': _w((lambda *s: _rng.normal(s) * 0.05)(Hq * Dh, D) * (Hq * Dh) ** (-0.5))}
    _A_in = _A_setup()

    def _B_setup():
        B, S, D, F = (1, 1, 640, 1536)
        return {'x': _w((lambda *s: _rng.normal(s) * 0.05)(B, S, D)), 'w_gate': _w((lambda *s: _rng.normal(s) * 0.05)(D, F)), 'w_up': _w((lambda *s: _rng.normal(s) * 0.05)(D, F)), 'w_down': _w((lambda *s: _rng.normal(s) * 0.05)(F, D))}
    _B_in = _B_setup()
    return {'A_x': _A_in['x'], 'A_k_cache': _A_in['k_cache'], 'A_v_cache': _A_in['v_cache'], 'A_wq': _A_in['wq'], 'A_wo': _A_in['wo'], 'B_x': _B_in['x'], 'B_w_gate': _B_in['w_gate'], 'B_w_up': _B_in['w_up'], 'B_w_down': _B_in['w_down'], 'c': _w((lambda *s: _rng.normal(s) * 0.05)(1, 640)), 'w_mod': _w((lambda *s: _rng.normal(s) * 0.05)(640, 6 * 640) * 640 ** (-0.5))}

def reference(A_x, A_k_cache, A_v_cache, A_wq, A_wo, B_x, B_w_gate, B_w_up, B_w_down, c, w_mod):

    def _A_ref(x, k_cache, v_cache, wq, wo):
        B, Sq, D = x.shape
        Hq, Dh = (32, 192)
        Hkv, Sk = (k_cache.shape[1], k_cache.shape[2])
        W = min(4096, max(256, Sk // 4))
        rep = Hq // Hkv
        q = (lambda x, *d: x.transpose(*d))((x @ wq).reshape(B, Sq, Hq, Dh), 0, 2, 1, 3)
        k = jnp.repeat(k_cache[:, :, Sk - W:, :], rep, axis=1)
        v = jnp.repeat(v_cache[:, :, Sk - W:, :], rep, axis=1)
        scores = jnp.einsum('bhqd,bhkd->bhqk', q, k) * Dh ** (-0.5)
        p = _softmax(scores, axis=-1)
        o = jnp.einsum('bhqk,bhkd->bhqd', p, v)
        return (lambda x, *d: x.transpose(*d))(o, 0, 2, 1, 3).reshape(B, Sq, Hq * Dh) @ wo

    def _B_ref(x, w_gate, w_up, w_down):
        return _gelu(x @ w_gate) * (x @ w_up) @ w_down
    x = A_x
    mod = (_silu(c) @ w_mod).reshape(c.shape[0], 6, 1, -1)
    sa, ca, ga, sb, cb, gb = (mod[:, 0].copy(), mod[:, 1].copy(), mod[:, 2].copy(), mod[:, 3].copy(), mod[:, 4].copy(), mod[:, 5].copy())
    h = _layernorm(x, axis=-1) * (1 + ca) + sa
    x = x + ga * _A_ref(h, A_k_cache, A_v_cache, A_wq, A_wo)
    h = _layernorm(x, axis=-1) * (1 + cb) + sb
    x = x + gb * _B_ref(h, B_w_gate, B_w_up, B_w_down)
    return x
```

```python
import functools
import math
import jax
import jax.numpy as jnp
from jax import lax
from jax.experimental import pallas as pl
from jax.experimental.pallas import tpu as pltpu

D = 640
H = 32
DH = 192
SK = 32768
W = 4096
F = 1536
NP = H // 2
PR = 2 * DH
EPS = 1e-5
F32 = jnp.float32
BF16 = jnp.bfloat16


def make_kernel(PU=1024, NB=4, M=8, KR=32, KC=512, pairing='rowhalf', name='adaln_v1', vmem_mb=100):
    NU = W // PU
    assert (2 * NU) % NB == 0 or NB % (2 * NU) == 0
    assert NB <= 2 * NU

    def kernel(x_hbm, k_hbm, v_hbm, wq_hbm, wo_hbm, wg_hbm, wu_hbm, wd_hbm, c_hbm, wm_hbm,
               o_hbm,
               ring, wq_b, wo_b, wm_b, wg_b, wu_b, wd_b, x_b, c_b, o_b,
               ring_sem, wq_sem, wo_sem, wm_sem, f_sem, m_sem):

        def start_many(copies):
            for i, (s, d, sem) in enumerate(copies):
                pltpu.make_async_copy(s, d, sem).start(priority=i % 2)

        def unit_copies(src, p, j, slot):
            r0 = p * PR
            p0 = SK - W + j * PU
            idx = [(r, c) for r in range(PR // KR) for c in range(PU // KC)]
            if pairing == 'rowhalf':
                n = len(idx)
                idx = [x for a, b in zip(idx[:n // 2], idx[n // 2:]) for x in (a, b)]
            out = []
            for r, c in idx:
                out.append((src.at[pl.ds(pl.multiple_of(r0 + r * KR, KR), KR), pl.ds(p0 + c * KC, KC)],
                            ring.at[slot, pl.ds(r * KR, KR), pl.ds(c * KC, KC)], ring_sem.at[slot]))
            return out

        def unit_wait(slot):
            pltpu.make_async_copy(ring.at[slot], ring.at[slot], ring_sem.at[slot]).wait()

        def tile_copies(src, dst, r0, nr, c0, nc, tr, tc, sem):
            out = []
            for r in range(nr // tr):
                for c in range(nc // tc):
                    rs = r0 + r * tr
                    cs = c0 + c * tc
                    if not isinstance(rs, int):
                        rs = pl.multiple_of(rs, tr if r0 is not None else 8)
                    if not isinstance(cs, int):
                        cs = pl.multiple_of(cs, 128)
                    out.append((src.at[pl.ds(rs, tr), pl.ds(cs, tc)], dst.at[pl.ds(rs, tr), pl.ds(cs, tc)], sem))
            return out

        def win_wait(dst, r0, nr, c0, nc, sem):
            if not isinstance(r0, int):
                r0 = pl.multiple_of(r0, 8)
            if not isinstance(c0, int):
                c0 = pl.multiple_of(c0, 128)
            v = dst.at[pl.ds(r0, nr), pl.ds(c0, nc)]
            pltpu.make_async_copy(v, v, sem).wait()

        def wq_copies(p):
            return tile_copies(wq_hbm, wq_b, 0, D, p * PR, PR, 40, PR, wq_sem.at[p % 2])

        def wq_wait(p):
            win_wait(wq_b, 0, D, p * PR, PR, wq_sem.at[p % 2])

        def wo_copies(p):
            return tile_copies(wo_hbm, wo_b, p * PR, PR, 0, D, 24, D, wo_sem.at[p % 2])

        def wo_wait(p):
            win_wait(wo_b, p * PR, PR, 0, D, wo_sem.at[p % 2])

        def wm_copies(i):
            return tile_copies(wm_hbm, wm_b, 0, D, i * D, D, 16, D, wm_sem.at[i])

        def wm_wait(i):
            win_wait(wm_b, 0, D, i * D, D, wm_sem.at[i])

        cx = pltpu.make_async_copy(c_hbm, c_b, m_sem.at[0])
        cx.start()
        xx = pltpu.make_async_copy(x_hbm, x_b, m_sem.at[1])
        xx.start()
        start_many(wm_copies(0))
        start_many(wm_copies(1))
        start_many(wq_copies(0))
        for s in range(NB):
            u = s
            src = k_hbm if u < NU else v_hbm
            start_many(unit_copies(src, 0, u % NU, s))

        def ln(v):
            m = jnp.mean(v, axis=-1, keepdims=True)
            d = v - m
            var = jnp.mean(d * d, axis=-1, keepdims=True)
            return d / jnp.sqrt(var + EPS)

        def bc(v):
            return jnp.broadcast_to(v, (M, v.shape[-1]))

        cx.wait()
        cs = c_b[...].astype(F32)
        cs = cs * jax.nn.sigmoid(cs)
        cs = bc(cs).astype(BF16)

        def mod_chunk(i):
            wm_wait(i)
            return jnp.dot(cs, wm_b[:, i * D:(i + 1) * D], preferred_element_type=F32)

        xx.wait()
        x0 = bc(x_b[...].astype(F32))
        sa = mod_chunk(0)
        ca = mod_chunk(1)
        h = (ln(x0) * (1.0 + ca) + sa).astype(BF16)

        row = lax.broadcasted_iota(jnp.int32, (M, PR), 0)
        col = lax.broadcasted_iota(jnp.int32, (M, PR), 1)
        dmask = row == (col // DH)
        scale = DH ** -0.5

        def ffn_part(i):
            if i == 0:
                return tile_copies(wg_hbm, wg_b, 0, D, 0, F, 8, F, f_sem.at[0])
            if i == 1:
                return tile_copies(wu_hbm, wu_b, 0, D, 0, F, 8, F, f_sem.at[1])
            if i == 2:
                return tile_copies(wd_hbm, wd_b, 0, F // 2, 0, D, 24, D, f_sem.at[2])
            if i == 3:
                return tile_copies(wd_hbm, wd_b, F // 2, F // 2, 0, D, 24, D, f_sem.at[3])
            return []

        n_tail_pts = NB

        def body(p, acc):
            wq_wait(p)
            q = jnp.dot(h, wq_b[:, pl.ds(pl.multiple_of(p * PR, 128), PR)], preferred_element_type=F32)
            q2 = jnp.where(dmask, q, 0.0).astype(BF16)

            def issue(u):
                slot = u % NB
                un = u + NB
                if un < 2 * NU:
                    src = k_hbm if un < NU else v_hbm
                    start_many(unit_copies(src, p, un % NU, slot))
                else:
                    un2 = un - 2 * NU
                    src = k_hbm if un2 < NU else v_hbm

                    @pl.when(p + 1 < NP)
                    def _():
                        start_many(unit_copies(src, p + 1, un2 % NU, slot))

                    ti = u - (2 * NU - NB)
                    parts = [i for i in range(4) if i * n_tail_pts // 4 == ti] if n_tail_pts < 4 else ([ti] if ti < 4 else [])
                    if parts:
                        @pl.when(p + 1 == NP)
                        def _():
                            for i in parts:
                                start_many(ffn_part(i))

            ss = []
            for j in range(NU):
                slot = j % NB
                unit_wait(slot)
                ss.append(jnp.dot(q2, ring[slot], preferred_element_type=F32))
                issue(j)
                if j == 0:
                    @pl.when(p + 1 < NP)
                    def _():
                        start_many(wq_copies(p + 1))
                if j == 1 % NU:
                    start_many(wo_copies(p))
                if j == NU - 1:
                    @pl.when(p < 4)
                    def _():
                        for i in range(4):
                            @pl.when(p == i)
                            def _():
                                start_many(wm_copies(2 + i))
            m = functools.reduce(jnp.maximum, ss)
            m = jnp.max(m, axis=-1, keepdims=True)
            es = [jnp.exp((s - m) * scale) for s in ss]
            l = jnp.sum(functools.reduce(jnp.add, es), axis=-1, keepdims=True)
            o = None
            for j in range(NU):
                slot = (NU + j) % NB
                unit_wait(slot)
                t = lax.dot_general(es[j].astype(BF16), ring[slot], (((1,), (1,)), ((), ())),
                                    preferred_element_type=F32)
                o = t if o is None else o + t
                issue(NU + j)
            on = jnp.where(dmask, o / l, 0.0).astype(BF16)
            wo_wait(p)
            acc = acc + jnp.dot(on, wo_b[pl.ds(pl.multiple_of(p * PR, PR), PR), :], preferred_element_type=F32)
            return acc

        acc = lax.fori_loop(0, NP, body, jnp.zeros((M, D), F32))

        ga = mod_chunk(2)
        sb = mod_chunk(3)
        cb = mod_chunk(4)
        gb = mod_chunk(5)
        attn = bc(jnp.sum(acc, axis=0, keepdims=True))
        x1 = x0 + ga * attn
        h2 = (ln(x1) * (1.0 + cb) + sb).astype(BF16)
        pltpu.make_async_copy(wg_b, wg_b, f_sem.at[0]).wait()
        g = jnp.dot(h2, wg_b[...], preferred_element_type=F32)
        pltpu.make_async_copy(wu_b, wu_b, f_sem.at[1]).wait()
        u = jnp.dot(h2, wu_b[...], preferred_element_type=F32)
        a = (jax.nn.gelu(g, approximate=True) * u).astype(BF16)
        FH = F // 2
        win_wait(wd_b, 0, FH, 0, D, f_sem.at[2])
        y = jnp.dot(a[:, :FH], wd_b[:FH, :], preferred_element_type=F32)
        win_wait(wd_b, FH, FH, 0, D, f_sem.at[3])
        y = y + jnp.dot(a[:, FH:], wd_b[FH:, :], preferred_element_type=F32)
        out = x1 + gb * y
        o_b[...] = out[:1].astype(BF16)
        oc = pltpu.make_async_copy(o_b, o_hbm, m_sem.at[2])
        oc.start()
        oc.wait()

    def fn(A_x, A_k_cache, A_v_cache, A_wq, A_wo, B_x, B_w_gate, B_w_up, B_w_down, c, w_mod):
        kt = jnp.swapaxes(A_k_cache, 2, 3).reshape(H * DH, SK)
        vt = jnp.swapaxes(A_v_cache, 2, 3).reshape(H * DH, SK)
        x2 = A_x.reshape(1, D)
        any_spec = pl.BlockSpec(memory_space=pl.ANY)
        out = pl.pallas_call(
            kernel,
            name=name,
            out_shape=jax.ShapeDtypeStruct((1, D), BF16),
            in_specs=[any_spec] * 10,
            out_specs=any_spec,
            scratch_shapes=[
                pltpu.VMEM((NB, PR, PU), BF16),
                pltpu.VMEM((D, H * DH), BF16),
                pltpu.VMEM((H * DH, D), BF16),
                pltpu.VMEM((D, 6 * D), BF16),
                pltpu.VMEM((D, F), BF16),
                pltpu.VMEM((D, F), BF16),
                pltpu.VMEM((F, D), BF16),
                pltpu.VMEM((1, D), BF16),
                pltpu.VMEM((1, D), BF16),
                pltpu.VMEM((1, D), BF16),
                pltpu.SemaphoreType.DMA((NB,)),
                pltpu.SemaphoreType.DMA((2,)),
                pltpu.SemaphoreType.DMA((2,)),
                pltpu.SemaphoreType.DMA((6,)),
                pltpu.SemaphoreType.DMA((4,)),
                pltpu.SemaphoreType.DMA((3,)),
            ],
            compiler_params=pltpu.CompilerParams(vmem_limit_bytes=vmem_mb * 1024 * 1024),
        )(x2, kt, vt, A_wq, A_wo, B_w_gate, B_w_up, B_w_down, c, w_mod)
        return out.reshape(1, 1, D)
    return fn


_fn = make_kernel(PU=512, NB=8)


@jax.jit
def pallas_adaLN_cond__sliding_block_cached__geglu_ffn__decode_kernel(
    A_x, A_k_cache, A_v_cache, A_wq, A_wo, B_x, B_w_gate, B_w_up, B_w_down, c, w_mod,
):
    return _fn(A_x, A_k_cache, A_v_cache, A_wq, A_wo, B_x, B_w_gate, B_w_up, B_w_down, c, w_mod)
```

```python
import functools
import jax
import jax.numpy as jnp
from jax import lax
from jax.experimental import pallas as pl
from jax.experimental.pallas import tpu as pltpu

D = 640
H = 32
DH = 192
SK = 32768
W = 4096
F = 1536
NP = H // 2
PR = 2 * DH
EPS = 1e-5
F32 = jnp.float32
BF16 = jnp.bfloat16
M = 8


def make_kernel(NB=6, UR=128, UP=2048, name='adaln_v2', vmem_mb=100, dmaonly=False,
                s_wm=16, s_wq=20, s_wo=16, s_wg=8, s_wd=8, nwd=2, ffn_pts=None, nochk=True, kvperm=1):
    KT = PR // UR
    NH = W // UP
    NU = KT * NH
    assert (2 * NU) % NB == 0
    CH = UR // 8

    def kernel(x_hbm, k_hbm, v_hbm, wq_hbm, wo_hbm, wg_hbm, wu_hbm, wd_hbm, c_hbm, wm_hbm,
               o_hbm,
               ring, wq_b, wo_b, wm_b, wg_b, wu_b, wd_b, x_b, c_b, o_b, tmp,
               ring_sem, w_sem, f_sem):

        def cp(src, dst, r0, nr, c0, nc, sem):
            if not isinstance(r0, int):
                r0 = pl.multiple_of(r0, 8)
            if not isinstance(c0, int):
                c0 = pl.multiple_of(c0, 128)
            return pltpu.make_async_copy(src.at[pl.ds(r0, nr), pl.ds(c0, nc)],
                                         dst.at[pl.ds(r0, nr), pl.ds(c0, nc)], sem)

        def wait_all(dst, r0, nr, sem):
            v = dst.at[pl.ds(r0, nr)]
            pltpu.make_async_copy(v, v, sem).wait()

        def stream(src, dst, tr, tc, s, sem, r_base=0, n_rows=None):
            n_rows = src.shape[0] - r_base if n_rows is None else n_rows
            ncol = src.shape[1] // tc
            n = (n_rows // tr) * ncol
            assert n_rows % tr == 0 and src.shape[1] % tc == 0 and n % s == 0 and (n // s) % 2 == 0

            def body(a, carry):
                for b in range(n // s):
                    idx = b * s + a
                    if ncol == 1:
                        r, c = idx, 0
                    elif s % ncol == 0:
                        r, c = b * (s // ncol) + a // ncol, a % ncol
                    else:
                        r, c = idx // ncol, idx % ncol
                    cp(src, dst, r_base + r * tr, tr, c * tc, tc, sem).start(priority=b % 2)
                return carry

            lax.fori_loop(0, s, body, 0)

        def unit_start(src, p, u, slot):
            r0 = p * PR + (u % KT) * UR
            c0 = SK - W + (u // KT) * UP
            for i in range(CH):
                j = (i * kvperm) % CH
                pltpu.make_async_copy(
                    src.at[pl.ds(pl.multiple_of(r0 + j * 8, 8), 8), pl.ds(c0, UP)],
                    ring.at[slot, pl.ds(j * 8, 8), :], ring_sem.at[slot]).start(priority=i % 2)

        def unit_wait(slot):
            pltpu.make_async_copy(ring.at[slot], ring.at[slot], ring_sem.at[slot]).wait()

        def ln(v):
            m = jnp.mean(v, axis=-1, keepdims=True)
            d = v - m
            var = jnp.mean(d * d, axis=-1, keepdims=True)
            return d / jnp.sqrt(var + EPS)

        def bc(v):
            return jnp.broadcast_to(v, (M, v.shape[-1]))

        c_cp = pltpu.make_async_copy(c_hbm, c_b, f_sem.at[0])
        c_cp.start(priority=0)
        x_cp = pltpu.make_async_copy(x_hbm, x_b, f_sem.at[1])
        x_cp.start(priority=1)
        stream(wm_hbm, wm_b, 8, 1920, s_wm, w_sem.at[0])
        stream(wq_hbm, wq_b, 8, 2048, s_wq, w_sem.at[1])

        c_cp.wait()
        x_cp.wait()
        wait_all(wm_b, 0, D, w_sem.at[0])
        if not dmaonly:
            cs = c_b[...].astype(F32)
            cs = bc(cs * jax.nn.sigmoid(cs)).astype(BF16)
            x0 = bc(x_b[...].astype(F32))
            mod = jnp.dot(cs, wm_b[...], preferred_element_type=F32)
            sa, ca = mod[:, 0:D], mod[:, D:2 * D]
            h = (ln(x0) * (1.0 + ca) + sa).astype(BF16)
            tmp[:, 0:4 * D] = mod[:, 2 * D:6 * D]
            tmp[:, 4 * D:5 * D] = x0

        stream(wo_hbm, wo_b, 24, D, s_wo, w_sem.at[2])

        def pro(s, carry):
            unit_start(k_hbm, 0, s, s)
            return carry
        for s in range(NB):
            unit_start(k_hbm if s < NU else v_hbm, 0, s % NU, s)

        wait_all(wq_b, 0, D, w_sem.at[1])
        wait_all(wo_b, 0, H * DH, w_sem.at[2])

        row = lax.broadcasted_iota(jnp.int32, (M, PR), 0)
        col = lax.broadcasted_iota(jnp.int32, (M, PR), 1)
        dmask = row == (col // DH)
        scale = DH ** -0.5
        FD = F // nwd

        def ffn_part(i):
            if i == 0:
                stream(wg_hbm, wg_b, 8, F, s_wg, f_sem.at[0])
            elif i == 1:
                stream(wu_hbm, wu_b, 8, F, s_wg, f_sem.at[1])
            else:
                stream(wd_hbm, wd_b, 24, D, s_wd, f_sem.at[i], r_base=(i - 2) * FD, n_rows=FD)

        nparts = 2 + nwd
        pts = ffn_pts if ffn_pts is not None else [i * NB // nparts for i in range(nparts)]

        def body(p, acc):
            def issue(u):
                slot = u % NB
                un = u + NB
                if un < 2 * NU:
                    unit_start(k_hbm if un < NU else v_hbm, p, un % NU, slot)
                else:
                    un2 = un - 2 * NU

                    @pl.when(p + 1 < NP)
                    def _():
                        unit_start(k_hbm if un2 < NU else v_hbm, p + 1, un2 % NU, slot)

                    ti = u - (2 * NU - NB)
                    parts = [i for i in range(nparts) if pts[i] == ti]
                    if parts:
                        @pl.when(p + 1 == NP)
                        def _():
                            for i in parts:
                                ffn_part(i)

            if not dmaonly:
                q = jnp.dot(h, wq_b[:, pl.ds(pl.multiple_of(p * PR, 128), PR)], preferred_element_type=F32)
                q2 = jnp.where(dmask, q, 0.0).astype(BF16)
            ss = [None] * NH
            for u in range(NU):
                slot = u % NB
                unit_wait(slot)
                if not dmaonly:
                    hf, kt = u // KT, u % KT
                    t = jnp.dot(q2[:, kt * UR:(kt + 1) * UR], ring[slot], preferred_element_type=F32)
                    ss[hf] = t if ss[hf] is None else ss[hf] + t
                issue(u)
            if not dmaonly:
                m = jnp.max(functools.reduce(jnp.maximum, ss), axis=-1, keepdims=True)
                es = [jnp.exp((s - m) * scale) for s in ss]
                l = jnp.sum(functools.reduce(jnp.add, es), axis=-1, keepdims=True)
                es = [e.astype(BF16) for e in es]
            os_ = [None] * KT
            for u in range(NU):
                slot = (NU + u) % NB
                unit_wait(slot)
                if not dmaonly:
                    hf, kt = u // KT, u % KT
                    t = lax.dot_general(es[hf], ring[slot], (((1,), (1,)), ((), ())), preferred_element_type=F32)
                    os_[kt] = t if os_[kt] is None else os_[kt] + t
                issue(NU + u)
            if dmaonly:
                return acc
            o = jnp.concatenate(os_, axis=1)
            on = jnp.where(dmask, o / l, 0.0).astype(BF16)
            return acc + jnp.dot(on, wo_b[pl.ds(pl.multiple_of(p * PR, PR), PR), :], preferred_element_type=F32)

        acc = lax.fori_loop(0, NP, body, jnp.zeros((M, D), F32))

        if not dmaonly:
            ga, sb, cb, gb, x0 = [tmp[:, i * D:(i + 1) * D] for i in range(5)]
            attn = bc(jnp.sum(acc, axis=0, keepdims=True))
            x1 = x0 + ga * attn
            h2 = (ln(x1) * (1.0 + cb) + sb).astype(BF16)
            tmp[:, 4 * D:5 * D] = x1
        wait_all(wg_b, 0, D, f_sem.at[0])
        if not dmaonly:
            g = jnp.dot(h2, wg_b[...], preferred_element_type=F32)
            tmp[:, 0:F] = jax.nn.gelu(g, approximate=True)
        wait_all(wu_b, 0, D, f_sem.at[1])
        if not dmaonly:
            u_ = jnp.dot(h2, wu_b[...], preferred_element_type=F32)
            a = (tmp[:, 0:F] * u_).astype(BF16)
        for i in range(nwd):
            wait_all(wd_b, i * FD, FD, f_sem.at[2 + i])
            if not dmaonly:
                t = jnp.dot(a[:, i * FD:(i + 1) * FD], wd_b[i * FD:(i + 1) * FD, :], preferred_element_type=F32)
                if i > 0:
                    t = t + tmp[:, 0:D]
                if i < nwd - 1:
                    tmp[:, 0:D] = t
        if not dmaonly:
            out = tmp[:, 4 * D:5 * D] + tmp[:, 3 * D:4 * D] * t
            o_b[...] = out[:1].astype(BF16)
        else:
            o_b[...] = x_b[...]
        oc = pltpu.make_async_copy(o_b, o_hbm, f_sem.at[0])
        oc.start()
        oc.wait()

    def fn(A_x, A_k_cache, A_v_cache, A_wq, A_wo, B_x, B_w_gate, B_w_up, B_w_down, c, w_mod):
        kt = jnp.swapaxes(A_k_cache, 2, 3).reshape(H * DH, SK)
        vt = jnp.swapaxes(A_v_cache, 2, 3).reshape(H * DH, SK)
        x2 = A_x.reshape(1, D)
        any_spec = pl.BlockSpec(memory_space=pl.ANY)
        out = pl.pallas_call(
            kernel,
            name=name,
            out_shape=jax.ShapeDtypeStruct((1, D), BF16),
            in_specs=[any_spec] * 10,
            out_specs=any_spec,
            scratch_shapes=[
                pltpu.VMEM((NB, UR, UP), BF16),
                pltpu.VMEM((D, H * DH), BF16),
                pltpu.VMEM((H * DH, D), BF16),
                pltpu.VMEM((D, 6 * D), BF16),
                pltpu.VMEM((D, F), BF16),
                pltpu.VMEM((D, F), BF16),
                pltpu.VMEM((F, D), BF16),
                pltpu.VMEM((1, D), BF16),
                pltpu.VMEM((1, D), BF16),
                pltpu.VMEM((1, D), BF16),
                pltpu.VMEM((M, 5 * D), F32),
                pltpu.SemaphoreType.DMA((NB,)),
                pltpu.SemaphoreType.DMA((3,)),
                pltpu.SemaphoreType.DMA((2 + nwd,)),
            ],
            compiler_params=pltpu.CompilerParams(vmem_limit_bytes=vmem_mb * 1024 * 1024,
                                                 disable_bounds_checks=nochk, disable_semaphore_checks=nochk),
        )(x2, kt, vt, A_wq, A_wo, B_w_gate, B_w_up, B_w_down, c, w_mod)
        return out.reshape(1, 1, D)
    return fn


_fn = make_kernel()


@jax.jit
def pallas_adaLN_cond__sliding_block_cached__geglu_ffn__decode_kernel(
    A_x, A_k_cache, A_v_cache, A_wq, A_wo, B_x, B_w_gate, B_w_up, B_w_down, c, w_mod,
):
    return _fn(A_x, A_k_cache, A_v_cache, A_wq, A_wo, B_x, B_w_gate, B_w_up, B_w_down, c, w_mod)
```

```python
import functools
import math
import jax
import jax.numpy as jnp
from jax import lax
from jax.experimental import pallas as pl
from jax.experimental.pallas import tpu as pltpu

D = 640
H = 32
DH = 192
SK = 32768
W = 4096
F = 1536
NP = H // 2
PR = 2 * DH
EPS = 1e-5
F32 = jnp.float32
BF16 = jnp.bfloat16
M = 8
CT = 16
KD = D // 128
KF = F // 128


def _tiles(w):
    r, c = w.shape
    return w.reshape(r // 8, 8, c // 128, 128).transpose(0, 2, 1, 3).reshape(r // 8 * (c // 128), 8, 128)


def make_kernel(name='adaln_v7', vmem_mb=100, dmaonly=False,
                o_wm=('half', 16, 8), o_wq=('st', 20, 0), o_wo=('st', 20, 0), o_wg=('half', 8, 0),
                o_wd=('half', 4, 0), wd_split=(6, 4, 2), pts=(0, 2, 6, 8, 8),
                mod_loop=False, pair_gu=False, xc_late=False, UR=128, UP=1024, CR=32, CP=512, NB=12):
    KT = PR // UR
    NH = W // UP
    NU = KT * NH
    assert (2 * NU) % NB == 0 and NB <= NU and len(pts) == 2 + len(wd_split)
    nwd = len(wd_split)
    assert sum(wd_split) == KF and len(pts) == 2 + nwd
    wd_off = [sum(wd_split[:i]) for i in range(nwd)]
    NT_M, NT_Q, NT_F = D // 8 * (6 * KD), D // 8 * (H * DH // 128), D // 8 * KF

    def kernel(x_hbm, k_hbm, v_hbm, wq_hbm, wo_hbm, wg_hbm, wu_hbm, wd_hbm, c_hbm, wm_hbm,
               o_hbm,
               ring, wq_b, wo_b, wm_b, wg_b, wu_b, wd_b, x_b, c_b, o_b,
               mod_s, g_s,
               ring_sem, w_sem, f_sem, d_sem):

        def loop(n, fn, init, unroll):
            if unroll:
                for i in range(n):
                    init = fn(i, init)
                return init
            return lax.fori_loop(0, n, fn, init)

        def chunk(src, dst, t, sem, prio, n=CT):
            pltpu.make_async_copy(src.at[pl.ds(t, n)], dst.at[pl.ds(t, n)], sem).start(priority=prio)

        def stream(src, dst, t0, nt, mode, s, phi, sem_of):
            n = (nt - phi) // CT
            n -= n % 2
            rem = nt - phi - n * CT
            if phi:
                chunk(src, dst, t0, sem_of(t0), 0, phi)
            if rem:
                chunk(src, dst, t0 + nt - rem, sem_of(t0 + nt - rem), 1, rem)
            base = t0 + phi
            span = n // 2 if mode == 'half' else n
            g = math.gcd(s, span)
            assert mode == 'half' or (span // g) % 2 == 0
            steps = span // g if mode == 'half' else span // g // 2

            def go(i, prio):
                t = base + i * CT
                chunk(src, dst, t, sem_of(t), prio)

            def nxt(i):
                i = i + s
                return jnp.where(i >= span, i - span, i)

            def inner(_, i):
                go(i, 0)
                if mode == 'half':
                    go(i + span, 1)
                else:
                    i = nxt(i)
                    go(i, 1)
                return nxt(i)

            def outer(cyc, carry):
                lax.fori_loop(0, steps, inner, cyc)
                return carry

            lax.fori_loop(0, g, outer, 0)

        def wait_tiles(dst, t0, nt, sem):
            v = dst.at[pl.ds(t0, nt)]
            pltpu.make_async_copy(v, v, sem).wait()

        def mm(lhs, buf, ncol, kb0, nkb, nb0, nnb):
            if not (isinstance(kb0, int) and isinstance(nb0, int)):
                buf = buf.at[pl.ds(16 * kb0 * ncol + nb0, (16 * nkb - 1) * ncol + nnb)]
                kb0 = nb0 = 0
            outs = []
            for nb in range(nnb):
                acc = None
                for kb in range(nkb):
                    w = buf[pl.ds(16 * (kb0 + kb) * ncol + nb0 + nb, 16, stride=ncol)].reshape(128, 128)
                    t = jnp.dot(lhs[:, kb * 128:(kb + 1) * 128], w, preferred_element_type=F32)
                    acc = t if acc is None else acc + t
                outs.append(acc)
            return outs[0] if nnb == 1 else jnp.concatenate(outs, axis=1)

        def unit_start(src, p, hf, kt, slot):
            r0 = p * PR + kt * UR
            c0 = SK - W + hf * UP
            i = 0
            for r in range(UR // CR):
                for c in range(UP // CP):
                    pltpu.make_async_copy(
                        src.at[pl.ds(pl.multiple_of(r0 + r * CR, 8), CR), pl.ds(c0 + c * CP, CP)],
                        ring.at[slot, pl.ds(r * CR, CR), pl.ds(c * CP, CP)], ring_sem.at[slot]).start(priority=i % 2)
                    i += 1

        def unit_wait(slot):
            pltpu.make_async_copy(ring.at[slot], ring.at[slot], ring_sem.at[slot]).wait()

        def ln(v):
            m = jnp.mean(v, axis=-1, keepdims=True)
            d = v - m
            var = jnp.mean(d * d, axis=-1, keepdims=True)
            return d / jnp.sqrt(var + EPS)

        def bc(v):
            return jnp.broadcast_to(v, (M, v.shape[-1]))

        c_cp = pltpu.make_async_copy(c_hbm, c_b, f_sem.at[0])
        x_cp = pltpu.make_async_copy(x_hbm, x_b, f_sem.at[1])
        if not xc_late:
            c_cp.start(priority=0)
            x_cp.start(priority=1)
        stream(wm_hbm, wm_b, 0, NT_M, *o_wm, lambda t: w_sem.at[0])
        if xc_late:
            c_cp.start(priority=0)
            x_cp.start(priority=1)
        stream(wq_hbm, wq_b, 0, NT_Q, *o_wq, lambda t: w_sem.at[1])

        c_cp.wait()
        x_cp.wait()
        wait_tiles(wm_b, 0, NT_M, w_sem.at[0])
        if not dmaonly:
            cs = c_b[...].astype(F32)
            cs = bc(cs * jax.nn.sigmoid(cs)).astype(BF16)

            def mod_body(i, carry):
                mod_s[i] = mm(cs, wm_b, 6 * KD, 0, KD, i * KD, KD)
                return carry
            loop(6, mod_body, 0, not mod_loop)
            x0 = bc(x_b[...].astype(F32))
            h = (ln(x0) * (1.0 + mod_s[1]) + mod_s[0]).astype(BF16)
            mod_s[0] = x0

        stream(wo_hbm, wo_b, 0, NT_Q, *o_wo, lambda t: w_sem.at[2])

        def pro(_, carry):
            for u in range(NB):
                unit_start(k_hbm, 0, u // KT, u % KT, u)
            return carry
        lax.fori_loop(0, 1, pro, 0)

        wait_tiles(wq_b, 0, NT_Q, w_sem.at[1])
        wait_tiles(wo_b, 0, NT_Q, w_sem.at[2])

        row3 = lax.broadcasted_iota(jnp.int32, (M, PR), 0)
        col3 = lax.broadcasted_iota(jnp.int32, (M, PR), 1)
        dmask = row3 == (col3 >= DH).astype(jnp.int32)
        scale = DH ** -0.5

        def ffn_part(i):
            if pair_gu and i < 2:
                if i == 0:
                    n, st = NT_F // CT, o_wg[1]
                    g = math.gcd(st, n)

                    def inner(_, j):
                        chunk(wg_hbm, wg_b, j * CT, f_sem.at[0], 0)
                        chunk(wu_hbm, wu_b, j * CT, f_sem.at[1], 1)
                        j = j + st
                        return jnp.where(j >= n, j - n, j)

                    def outer(cyc, carry):
                        lax.fori_loop(0, n // g, inner, cyc)
                        return carry
                    lax.fori_loop(0, g, outer, 0)
            elif i == 0:
                stream(wg_hbm, wg_b, 0, NT_F, *o_wg, lambda t: f_sem.at[0])
            elif i == 1:
                stream(wu_hbm, wu_b, 0, NT_F, *o_wg, lambda t: f_sem.at[1])
            else:
                j = i - 2
                t0, nt = wd_off[j] * 16 * KD, wd_split[j] * 16 * KD
                stream(wd_hbm, wd_b, t0, nt, *o_wd, lambda t: d_sem.at[j])

        def body(p, acc):
            if not dmaonly:
                q = mm(h, wq_b, H * DH // 128, 0, KD, p * KT, KT)
                q2 = jnp.where(dmask, q, 0.0).astype(BF16)
            def refill(g):
                slot, n = g % NB, g + NB
                if n < 2 * NU:
                    u = n % NU
                    unit_start(k_hbm if n < NU else v_hbm, p, u // KT, u % KT, slot)
                else:
                    u = n - 2 * NU
                    nxt = (k_hbm if u < NU else v_hbm, (u % NU) // KT, (u % NU) % KT)

                    @pl.when(p + 1 < NP)
                    def _():
                        unit_start(nxt[0], p + 1, nxt[1], nxt[2], slot)

                    parts = [i for i in range(2 + nwd) if pts[i] == g - (2 * NU - NB)]
                    if parts:
                        @pl.when(p + 1 == NP)
                        def _():
                            for i in parts:
                                ffn_part(i)

            ss = [None] * NH
            for u in range(NU):
                hf, kt = u // KT, u % KT
                unit_wait(u % NB)
                if not dmaonly:
                    t = jnp.dot(q2[:, kt * UR:(kt + 1) * UR], ring[u % NB], preferred_element_type=F32)
                    ss[hf] = t if ss[hf] is None else ss[hf] + t
                refill(u)
            if not dmaonly:
                m = jnp.max(functools.reduce(jnp.maximum, ss), axis=-1, keepdims=True)
                es = [jnp.exp((s - m) * scale) for s in ss]
                l = jnp.sum(functools.reduce(jnp.add, es), axis=-1, keepdims=True)
                es = [e.astype(BF16) for e in es]
            os_ = [None] * KT
            for u in range(NU):
                hf, kt = u // KT, u % KT
                unit_wait((NU + u) % NB)
                if not dmaonly:
                    t = lax.dot_general(es[hf], ring[(NU + u) % NB], (((1,), (1,)), ((), ())),
                                        preferred_element_type=F32)
                    os_[kt] = t if os_[kt] is None else os_[kt] + t
                refill(NU + u)
            if dmaonly:
                return acc
            on = jnp.where(dmask, jnp.concatenate(os_, axis=1) / l, 0.0).astype(BF16)
            return acc + mm(on, wo_b, KD, p * KT, KT, 0, KD)

        acc = lax.fori_loop(0, NP, body, jnp.zeros((M, D), F32))

        if not dmaonly:
            attn = bc(jnp.sum(acc, axis=0, keepdims=True))
            x1 = mod_s[0] + mod_s[2] * attn
            h2 = (ln(x1) * (1.0 + mod_s[4]) + mod_s[3]).astype(BF16)
            mod_s[0] = x1
        wait_tiles(wg_b, 0, NT_F, f_sem.at[0])
        if not dmaonly:
            g_s[...] = jax.nn.gelu(mm(h2, wg_b, KF, 0, KD, 0, KF), approximate=True)
        wait_tiles(wu_b, 0, NT_F, f_sem.at[1])
        if not dmaonly:
            a = (g_s[...] * mm(h2, wu_b, KF, 0, KD, 0, KF)).astype(BF16)
        for i in range(nwd):
            k0, n = wd_off[i], wd_split[i]
            wait_tiles(wd_b, k0 * 16 * KD, n * 16 * KD, d_sem.at[i])
            if not dmaonly:
                y = mm(a[:, k0 * 128:(k0 + n) * 128], wd_b, KD, k0, n, 0, KD)
                if i > 0:
                    y = y + mod_s[1]
                if i < nwd - 1:
                    mod_s[1] = y
        if not dmaonly:
            out = mod_s[0] + mod_s[5] * y
            o_b[...] = out[:1].astype(BF16)
        else:
            o_b[...] = x_b[...]
        oc = pltpu.make_async_copy(o_b, o_hbm, f_sem.at[0])
        oc.start()
        oc.wait()

    def fn(A_x, A_k_cache, A_v_cache, A_wq, A_wo, B_x, B_w_gate, B_w_up, B_w_down, c, w_mod):
        del B_x
        kt = jnp.swapaxes(A_k_cache, 2, 3).reshape(H * DH, SK)
        vt = jnp.swapaxes(A_v_cache, 2, 3).reshape(H * DH, SK)
        wq, wo, wg, wu, wd, wm = [_tiles(w) for w in (A_wq, A_wo, B_w_gate, B_w_up, B_w_down, w_mod)]
        any_spec = pl.BlockSpec(memory_space=pl.ANY)
        tb = lambda t: pltpu.VMEM(t.shape, BF16)
        out = pl.pallas_call(
            kernel,
            name=name,
            out_shape=jax.ShapeDtypeStruct((1, D), BF16),
            in_specs=[any_spec] * 10,
            out_specs=any_spec,
            scratch_shapes=[
                pltpu.VMEM((NB, UR, UP), BF16),
                tb(wq), tb(wo), tb(wm), tb(wg), tb(wu), tb(wd),
                pltpu.VMEM((1, D), BF16),
                pltpu.VMEM((1, D), BF16),
                pltpu.VMEM((1, D), BF16),
                pltpu.VMEM((6, M, D), F32),
                pltpu.VMEM((M, F), F32),
                pltpu.SemaphoreType.DMA((NB,)),
                pltpu.SemaphoreType.DMA((3,)),
                pltpu.SemaphoreType.DMA((2,)),
                pltpu.SemaphoreType.DMA((nwd,)),
            ],
            compiler_params=pltpu.CompilerParams(vmem_limit_bytes=vmem_mb * 1024 * 1024,
                                                 disable_bounds_checks=True, disable_semaphore_checks=True),
        )(A_x.reshape(1, D), kt, vt, wq, wo, wg, wu, wd, c, wm)
        return out.reshape(1, 1, D)
    return fn


_fn = make_kernel()


@jax.jit
def pallas_adaLN_cond__sliding_block_cached__geglu_ffn__decode_kernel(
    A_x, A_k_cache, A_v_cache, A_wq, A_wo, B_x, B_w_gate, B_w_up, B_w_down, c, w_mod,
):
    return _fn(A_x, A_k_cache, A_v_cache, A_wq, A_wo, B_x, B_w_gate, B_w_up, B_w_down, c, w_mod)
```

```python
import functools
import math

import jax
import jax.numpy as jnp
from jax import lax
from jax.experimental import pallas as pl
from jax.experimental.pallas import tpu as pltpu

D = 640
H = 32
DH = 192
SK = 32768
W = 4096
F = 1536
EPS = 1e-5
F32 = jnp.float32
BF16 = jnp.bfloat16

M = 8
HG = 4
NG = H // HG
GR = HG * DH
UR, UP = 128, 1024
CR, CP = 32, 512
KT = GR // UR
NH = W // UP
NU = KT * NH
NB = 12
CT = 16
KD = D // 128
KF = F // 128
WD_SPLIT = (6, 4, 2)
FFN_POINTS = (0, 2, 6, 8, 8)

ORDER_WM = ("half", 16, 8)
ORDER_WQ = ("alt", 20, 0)
ORDER_WO = ("alt", 20, 0)
ORDER_WGU = ("half", 8, 0)
ORDER_WD = ("half", 4, 0)


def _tiles(w):
    r, c = w.shape
    return w.reshape(r // 8, 8, c // 128, 128).transpose(0, 2, 1, 3).reshape(r // 8 * (c // 128), 8, 128)


def _layernorm(v):
    m = jnp.mean(v, axis=-1, keepdims=True)
    d = v - m
    var = jnp.mean(d * d, axis=-1, keepdims=True)
    return d / jnp.sqrt(var + EPS)


def _rows(v):
    return jnp.broadcast_to(v, (M, v.shape[-1]))


def _kernel(x_hbm, k_hbm, v_hbm, wq_hbm, wo_hbm, wg_hbm, wu_hbm, wd_hbm, c_hbm, wm_hbm,
            o_hbm,
            ring, wq_b, wo_b, wm_b, wg_b, wu_b, wd_b, x_b, c_b, o_b, mod_s, g_s,
            ring_sem, w_sem, f_sem, d_sem):
    nt_m, nt_q, nt_f = wm_b.shape[0], wq_b.shape[0], wg_b.shape[0]
    wd_off = [sum(WD_SPLIT[:i]) for i in range(len(WD_SPLIT))]

    def chunk(src, dst, t, sem, prio, n=CT):
        pltpu.make_async_copy(src.at[pl.ds(t, n)], dst.at[pl.ds(t, n)], sem).start(priority=prio)

    def stream(src, dst, t0, nt, order, sem):
        mode, s, phase = order
        n = (nt - phase) // CT
        n -= n % 2
        rem = nt - phase - n * CT
        if phase:
            chunk(src, dst, t0, sem, 0, phase)
        if rem:
            chunk(src, dst, t0 + nt - rem, sem, 1, rem)
        base = t0 + phase
        span = n // 2 if mode == "half" else n
        cycles = math.gcd(s, span)
        assert mode == "half" or (span // cycles) % 2 == 0
        steps = span // cycles if mode == "half" else span // cycles // 2

        def nxt(i):
            i = i + s
            return jnp.where(i >= span, i - span, i)

        def inner(_, i):
            chunk(src, dst, base + i * CT, sem, 0)
            if mode == "half":
                chunk(src, dst, base + (i + span) * CT, sem, 1)
            else:
                i = nxt(i)
                chunk(src, dst, base + i * CT, sem, 1)
            return nxt(i)

        def outer(cyc, carry):
            lax.fori_loop(0, steps, inner, cyc)
            return carry

        lax.fori_loop(0, cycles, outer, 0)

    def wait_tiles(dst, t0, nt, sem):
        v = dst.at[pl.ds(t0, nt)]
        pltpu.make_async_copy(v, v, sem).wait()

    def mm(lhs, buf, ncol, kb0, nkb, nb0, nnb):
        if not (isinstance(kb0, int) and isinstance(nb0, int)):
            buf = buf.at[pl.ds(16 * kb0 * ncol + nb0, (16 * nkb - 1) * ncol + nnb)]
            kb0 = nb0 = 0
        outs = []
        for nb in range(nb0, nb0 + nnb):
            acc = None
            for kb in range(nkb):
                w = buf[pl.ds(16 * (kb0 + kb) * ncol + nb, 16, stride=ncol)].reshape(128, 128)
                t = jnp.dot(lhs[:, kb * 128:(kb + 1) * 128], w, preferred_element_type=F32)
                acc = t if acc is None else acc + t
            outs.append(acc)
        return outs[0] if nnb == 1 else jnp.concatenate(outs, axis=1)

    def unit_start(src, g, u, slot):
        r0 = g * GR + (u % KT) * UR
        c0 = SK - W + (u // KT) * UP
        i = 0
        for r in range(UR // CR):
            for c in range(UP // CP):
                pltpu.make_async_copy(
                    src.at[pl.ds(pl.multiple_of(r0 + r * CR, CR), CR), pl.ds(c0 + c * CP, CP)],
                    ring.at[slot, pl.ds(r * CR, CR), pl.ds(c * CP, CP)],
                    ring_sem.at[slot]).start(priority=i % 2)
                i += 1

    def unit_wait(slot):
        pltpu.make_async_copy(ring.at[slot], ring.at[slot], ring_sem.at[slot]).wait()

    def ffn_start(i):
        if i == 0:
            stream(wg_hbm, wg_b, 0, nt_f, ORDER_WGU, f_sem.at[0])
        elif i == 1:
            stream(wu_hbm, wu_b, 0, nt_f, ORDER_WGU, f_sem.at[1])
        else:
            j = i - 2
            stream(wd_hbm, wd_b, wd_off[j] * 16 * KD, WD_SPLIT[j] * 16 * KD, ORDER_WD, d_sem.at[j])

    c_cp = pltpu.make_async_copy(c_hbm, c_b, f_sem.at[0])
    x_cp = pltpu.make_async_copy(x_hbm, x_b, f_sem.at[1])
    c_cp.start(priority=0)
    x_cp.start(priority=1)
    stream(wm_hbm, wm_b, 0, nt_m, ORDER_WM, w_sem.at[0])
    stream(wq_hbm, wq_b, 0, nt_q, ORDER_WQ, w_sem.at[1])

    c_cp.wait()
    x_cp.wait()
    wait_tiles(wm_b, 0, nt_m, w_sem.at[0])
    cs = c_b[...].astype(F32)
    cs = _rows(cs * jax.nn.sigmoid(cs)).astype(BF16)
    for i in range(6):
        mod_s[i] = mm(cs, wm_b, 6 * KD, 0, KD, i * KD, KD)
    x0 = _rows(x_b[...].astype(F32))
    h = (_layernorm(x0) * (1.0 + mod_s[1]) + mod_s[0]).astype(BF16)
    mod_s[0] = x0

    stream(wo_hbm, wo_b, 0, nt_q, ORDER_WO, w_sem.at[2])

    def fill_ring(_, carry):
        for u in range(NB):
            unit_start(k_hbm, 0, u, u)
        return carry

    lax.fori_loop(0, 1, fill_ring, 0)
    wait_tiles(wq_b, 0, nt_q, w_sem.at[1])
    wait_tiles(wo_b, 0, nt_q, w_sem.at[2])

    row = lax.broadcasted_iota(jnp.int32, (M, GR), 0)
    col = lax.broadcasted_iota(jnp.int32, (M, GR), 1)
    head = functools.reduce(jnp.add, [(col >= i * DH).astype(jnp.int32) for i in range(1, HG)])
    own = row == head
    scale = DH ** -0.5

    def step(g, acc):
        def refill(n):
            slot, nn = n % NB, n + NB
            if nn < 2 * NU:
                unit_start(k_hbm if nn < NU else v_hbm, g, nn % NU, slot)
                return

            @pl.when(g + 1 < NG)
            def _():
                unit_start(k_hbm, g + 1, nn - 2 * NU, slot)

            parts = [i for i, pt in enumerate(FFN_POINTS) if pt == n - (2 * NU - NB)]
            if parts:
                @pl.when(g + 1 == NG)
                def _():
                    for i in parts:
                        ffn_start(i)

        q = mm(h, wq_b, H * DH // 128, 0, KD, g * KT, KT)
        qd = jnp.where(own, q, 0.0).astype(BF16)

        scores = [None] * NH
        for u in range(NU):
            hf, kt = u // KT, u % KT
            unit_wait(u % NB)
            t = jnp.dot(qd[:, kt * UR:(kt + 1) * UR], ring[u % NB], preferred_element_type=F32)
            scores[hf] = t if scores[hf] is None else scores[hf] + t
            refill(u)

        mx = jnp.max(functools.reduce(jnp.maximum, scores), axis=-1, keepdims=True)
        es = [jnp.exp((s - mx) * scale) for s in scores]
        denom = jnp.sum(functools.reduce(jnp.add, es), axis=-1, keepdims=True)
        es = [e.astype(BF16) for e in es]

        outs = [None] * KT
        for u in range(NU):
            hf, kt = u // KT, u % KT
            slot = (NU + u) % NB
            unit_wait(slot)
            t = lax.dot_general(es[hf], ring[slot], (((1,), (1,)), ((), ())), preferred_element_type=F32)
            outs[kt] = t if outs[kt] is None else outs[kt] + t
            refill(NU + u)

        o = jnp.where(own, jnp.concatenate(outs, axis=1) / denom, 0.0).astype(BF16)
        return acc + mm(o, wo_b, KD, g * KT, KT, 0, KD)

    acc = lax.fori_loop(0, NG, step, jnp.zeros((M, D), F32))

    attn = _rows(jnp.sum(acc, axis=0, keepdims=True))
    x1 = mod_s[0] + mod_s[2] * attn
    h2 = (_layernorm(x1) * (1.0 + mod_s[4]) + mod_s[3]).astype(BF16)
    mod_s[0] = x1

    wait_tiles(wg_b, 0, nt_f, f_sem.at[0])
    g_s[...] = jax.nn.gelu(mm(h2, wg_b, KF, 0, KD, 0, KF), approximate=True)
    wait_tiles(wu_b, 0, nt_f, f_sem.at[1])
    a = (g_s[...] * mm(h2, wu_b, KF, 0, KD, 0, KF)).astype(BF16)

    y = None
    for i, (k0, n) in enumerate(zip(wd_off, WD_SPLIT)):
        if y is not None:
            mod_s[1] = y
        wait_tiles(wd_b, k0 * 16 * KD, n * 16 * KD, d_sem.at[i])
        t = mm(a[:, k0 * 128:(k0 + n) * 128], wd_b, KD, k0, n, 0, KD)
        y = t if y is None else t + mod_s[1]

    out = mod_s[0] + mod_s[5] * y
    o_b[...] = out[:1].astype(BF16)
    o_cp = pltpu.make_async_copy(o_b, o_hbm, f_sem.at[0])
    o_cp.start()
    o_cp.wait()


@jax.jit
def pallas_adaLN_cond__sliding_block_cached__geglu_ffn__decode_kernel(
    A_x: jax.Array,
    A_k_cache: jax.Array,
    A_v_cache: jax.Array,
    A_wq: jax.Array,
    A_wo: jax.Array,
    B_x: jax.Array,
    B_w_gate: jax.Array,
    B_w_up: jax.Array,
    B_w_down: jax.Array,
    c: jax.Array,
    w_mod: jax.Array,
):
    del B_x
    assert A_k_cache.shape == A_v_cache.shape == (1, H, SK, DH) and A_x.shape == (1, 1, D)
    kt = jnp.swapaxes(A_k_cache, 2, 3).reshape(H * DH, SK)
    vt = jnp.swapaxes(A_v_cache, 2, 3).reshape(H * DH, SK)
    wq, wo, wg, wu, wd, wm = [_tiles(w) for w in (A_wq, A_wo, B_w_gate, B_w_up, B_w_down, w_mod)]
    in_hbm = pl.BlockSpec(memory_space=pl.ANY)
    out = pl.pallas_call(
        _kernel,
        out_shape=jax.ShapeDtypeStruct((1, D), A_x.dtype),
        in_specs=[in_hbm] * 10,
        out_specs=in_hbm,
        scratch_shapes=[
            pltpu.VMEM((NB, UR, UP), BF16),
            *[pltpu.VMEM(t.shape, BF16) for t in (wq, wo, wm, wg, wu, wd)],
            pltpu.VMEM((1, D), BF16),
            pltpu.VMEM((1, D), BF16),
            pltpu.VMEM((1, D), BF16),
            pltpu.VMEM((6, M, D), F32),
            pltpu.VMEM((M, F), F32),
            pltpu.SemaphoreType.DMA((NB,)),
            pltpu.SemaphoreType.DMA((3,)),
            pltpu.SemaphoreType.DMA((2,)),
            pltpu.SemaphoreType.DMA((len(WD_SPLIT),)),
        ],
        compiler_params=pltpu.CompilerParams(
            vmem_limit_bytes=64 * 1024 * 1024,
            disable_semaphore_checks=True,
        ),
    )(A_x.reshape(1, D), kt, vt, wq, wo, wg, wu, wd, c, wm)
    return out.reshape(1, 1, D)
```
